```python
import jax
import jax.numpy as jnp

def _softmax(x, axis=-1):
    return jax.nn.softmax(x, axis=axis)

def _gelu(x):
    return jax.nn.gelu(x, approximate=True)

def _silu(x):
    return jax.nn.silu(x)

def _sigmoid(x):
    return jax.nn.sigmoid(x)

def _layernorm(x, axis=-1, eps=1e-05):
    m = jnp.mean(x, axis=axis, keepdims=True)
    v = jnp.var(x, axis=axis, keepdims=True)
    return (x - m) / jnp.sqrt(v + eps)

def _scatter_add(tgt, idx, src, axis=0):
    return tgt.at[idx].add(src)

def _segment_sum(src, seg, n):
    return jax.ops.segment_sum(src, seg, n)

class _Rng:

    def __init__(self, key):
        self._k = key

    def _next(self):
        self._k, sub = jax.random.split(self._k)
        return sub

    def normal(self, shape):
        return jax.random.normal(self._next(), shape, dtype=jnp.bfloat16)

    def randint(self, lo, hi, shape):
        return jax.random.randint(self._next(), shape, lo, hi, dtype=jnp.int32)

    def uniform(self, shape, lo=0.0, hi=1.0):
        return jax.random.uniform(self._next(), shape, jnp.bfloat16, lo, hi)

    def permutation(self, n):
        return jax.random.permutation(self._next(), n)
kernel_name = 'gated_mix__memory_aug_recurrent_mem_tr__ssm_conv_h3__prompt'

def setup_inputs():
    _rng = _Rng(jax.random.key(int.from_bytes(__import__("os").urandom(4), "little")))
    _w = lambda a: (lambda t: t.astype(jnp.bfloat16) if jnp.issubdtype(t.dtype, jnp.floating) else t)(jnp.asarray(a))

    def _A_setup():
        B, S, Dm = (1, 2048, 640)
        H, Dh = (32, 192)
        M, seg = (8, 32)
        seg = min(seg, S)
        S = S // seg * seg
        return {'x': _w((lambda *s: _rng.normal(s) * 0.05)(B, S, Dm)), 'mem0': _w((lambda *s: _rng.normal(s) * 0.05)(B, M, Dm)), 'Wq': _w((lambda *s: _rng.normal(s) * 0.05)(Dm, H, Dh) * Dm ** (-0.5)), 'Wk': _w((lambda *s: _rng.normal(s) * 0.05)(Dm, H, Dh) * Dm ** (-0.5)), 'Wv': _w((lambda *s: _rng.normal(s) * 0.05)(Dm, H, Dh) * Dm ** (-0.5)), 'Wo': _w((lambda *s: _rng.normal(s) * 0.05)(H, Dh, Dm) * (H * Dh) ** (-0.5)), 'seg_len': seg}
    _A_in = _A_setup()

    def _B_setup():
        B, S, D = (1, 2048, 640)
        ks = 4
        return {'q': _w((lambda *s: _rng.normal(s) * 0.05)(B, S, D)), 'k': _w((lambda *s: _rng.normal(s) * 0.05)(B, S, D)), 'v': _w((lambda *s: _rng.normal(s) * 0.05)(B, S, D)), 'shift_k': _w((lambda *s: _rng.normal(s) * 0.05)(D, ks) * 0.5), 'ssm_k': _w((lambda *s: _rng.normal(s) * 0.05)(D, S) * (1.0 / S ** 0.5)), 'ssm_D': _w((lambda *s: _rng.normal(s) * 0.05)(D))}
    _B_in = _B_setup()
    return {'A_x': _A_in['x'], 'A_mem0': _A_in['mem0'], 'A_Wq': _A_in['Wq'], 'A_Wk': _A_in['Wk'], 'A_Wv': _A_in['Wv'], 'A_Wo': _A_in['Wo'], 'A_seg_len': _A_in['seg_len'], 'B_q': _B_in['q'], 'B_k': _B_in['k'], 'B_v': _B_in['v'], 'B_shift_k': _B_in['shift_k'], 'B_ssm_k': _B_in['ssm_k'], 'B_ssm_D': _B_in['ssm_D'], 'gate_w': _w((lambda *s: _rng.normal(s) * 0.05)(640))}

def reference(A_x, A_mem0, A_Wq, A_Wk, A_Wv, A_Wo, A_seg_len, B_q, B_k, B_v, B_shift_k, B_ssm_k, B_ssm_D, gate_w):

    def _A_ref(x, mem0, Wq, Wk, Wv, Wo, seg_len):
        B, S, Dm = x.shape
        H, Dh = (Wq.shape[1], Wq.shape[2])
        M = mem0.shape[1]
        scale = Dh ** (-0.5)
        n_seg = S // seg_len
        L = M + seg_len
        idx = jnp.arange(L)
        mask = (idx[:, None] < M) | (idx[:, None] >= idx[None, :])
        mem = mem0
        outs = []
        for s in range(n_seg):
            xs = x[:, s * seg_len:(s + 1) * seg_len, :].copy()
            h = jnp.concatenate([mem, xs], axis=1)
            q = jnp.einsum('btd,dhe->bhte', h, Wq)
            k = jnp.einsum('btd,dhe->bhte', h, Wk)
            v = jnp.einsum('btd,dhe->bhte', h, Wv)
            scores = jnp.einsum('bhqe,bhke->bhqk', q, k) * scale
            scores = jnp.where(mask[None, None], scores, -1000000000.0)
            p = _softmax(scores, axis=-1)
            o = jnp.einsum('bhqk,bhke->bhqe', p, v)
            o = jnp.einsum('bhte,hed->btd', o, Wo)
            mem = o[:, :M, :].copy()
            outs.append(o[:, M:, :])
        return jnp.concatenate(outs, axis=1)

    def _B_ref(q, k, v, shift_k, ssm_k, ssm_D):
        B, S, D = q.shape
        ks = shift_k.shape[-1]
        k_pad = jnp.pad(k, ((0, 0), (ks - 1, 0), (0, 0)))
        k_shift = jnp.zeros_like(k)
        for t in range(ks):
            k_shift = k_shift + k_pad[:, t:t + S, :] * shift_k[:, ks - 1 - t][None, None, :]
        kv = k_shift * v
        L = 2 * S
        kv_pad = jnp.pad(kv, ((0, 0), (0, S), (0, 0)))
        kf_pad = jnp.pad(ssm_k, ((0, 0), (0, S)))
        kv_f = (lambda x, axes=(-2, -1): jnp.fft.rfft2(x.astype(jnp.float32), axes=axes))(kv_pad[:, None, :, :], axes=(1, 2))
        kf_f = (lambda x, axes=(-2, -1): jnp.fft.rfft2(x.astype(jnp.float32), axes=axes))(kf_pad[:, None, :], axes=(1, 2))
        kf_f = (lambda x, *d: x.transpose(*d))(kf_f, 1, 2, 0)
        y_f = kv_f * kf_f[None, :, :, :]
        y = (lambda x, s, axes=(-2, -1): jnp.fft.irfft2(x, s=s, axes=axes).astype(jnp.bfloat16))(y_f, (1, L), axes=(1, 2))[:, 0, :S, :]
        y = y + kv * ssm_D[None, None, :]
        return q * y
    x = A_x
    g = _sigmoid((x * gate_w).sum(-1, keepdims=True))
    a = _A_ref(x, A_mem0, A_Wq, A_Wk, A_Wv, A_Wo, A_seg_len)
    b = _B_ref(x, B_k, B_v, B_shift_k, B_ssm_k, B_ssm_D)
    return g * a + (1 - g) * b
```

```python
import functools

import jax
import jax.numpy as jnp
import numpy as np
from jax import lax
import jax.experimental.pallas as pl
import jax.experimental.pallas.tpu as pltpu

LANES = 128
CHUNK = 128
W_DMA_CHUNKS = 4

LAG_S, LAG_PV, LAG_O = 1, 2, 3

_F32 = jnp.float32
_BF16 = jnp.bfloat16
_NT = (((1,), (1,)), ((), ()))


def _dft_constants():
    w = np.pi * (np.arange(CHUNK, dtype=np.float64) + 0.5) / CHUNK
    t = np.arange(CHUNK, dtype=np.float64)
    ang = w[:, None] * t[None, :]
    fwd = np.concatenate([np.cos(ang), -np.sin(ang)], axis=0)
    inv = np.concatenate([np.cos(ang.T), -np.sin(ang.T)], axis=1) / CHUNK
    return fwd.astype(np.float32), inv.astype(np.float32)


def _kernel(
    x_hbm, mem0_ref, wq_hbm, wk_hbm, wv_hbm, wo_hbm, k_hbm, v_hbm,
    shift_ref, ssmk_hbm, ssmd_ref, gate_ref, fwd_ref, inv_ref,
    out_hbm,
    x_s, k_s, v_s, ssmk_s, wt_s, w_s, wo_s, kf_s, xh_s, kh_s, yh_s, b_s, out_s,
    in_sem, w_sem, wo_sem, out_sem,
    *, seg, n_mem, n_heads, d_head,
):
    seq = x_s.shape[1]
    n_ct = x_s.shape[0]
    d_model = n_ct * LANES
    n_chunks = seq // CHUNK
    n_seg = seq // seg
    rows = seg + n_mem
    n_pairs = n_heads // 2
    pair_w = 2 * d_head
    pair_t = pair_w // LANES
    n_wt = n_pairs * pair_t
    scale = float(d_head) ** -0.5
    n_taps = shift_ref.shape[0]

    def act_copies(c):
        cols = pl.ds(c * LANES, LANES)
        return (
            pltpu.make_async_copy(k_hbm.at[:, cols], k_s.at[c], in_sem.at[0, c]),
            pltpu.make_async_copy(v_hbm.at[:, cols], v_s.at[c], in_sem.at[1, c]),
            pltpu.make_async_copy(ssmk_hbm.at[cols, :], ssmk_s.at[c], in_sem.at[2, c]),
            pltpu.make_async_copy(x_hbm.at[:, cols], x_s.at[c], in_sem.at[3, c]),
        )

    w_rows = n_wt * LANES // W_DMA_CHUNKS

    def w_copy(m, j):
        src = (wq_hbm, wk_hbm, wv_hbm)[m]
        r = pl.ds(j * w_rows, w_rows)
        return pltpu.make_async_copy(src.at[r, :], wt_s.at[m, r, :], w_sem.at[m, j])

    def wo_copy(c):
        cols = pl.ds(c * LANES, LANES)
        return pltpu.make_async_copy(wo_hbm.at[:, cols], wo_s.at[c], wo_sem.at[c])

    for c in range(n_ct):
        for cp in act_copies(c):
            cp.start()
    for j in range(W_DMA_CHUNKS):
        for m in range(3):
            w_copy(m, j).start()
    for c in range(n_ct):
        wo_copy(c).start()

    kf_s[0:8, :] = jnp.zeros((8, LANES), _F32)
    fwd = fwd_ref[...]
    inv = inv_ref[...]
    sub = lax.broadcasted_iota(jnp.int32, (8, LANES), 0)
    sign = jnp.where(sub % 2 == 0, 1.0, -1.0).astype(_F32)

    for c in range(n_ct):
        for cp in act_copies(c):
            cp.wait()
        cols = slice(c * LANES, (c + 1) * LANES)
        taps = shift_ref[:, cols].astype(_F32)
        ssm_d = ssmd_ref[:, cols].astype(_F32)
        kf_s[8:, :] = k_s[c].astype(_F32)

        def fwd_chunk(j, carry, c=c, taps=taps, ssm_d=ssm_d):
            r0 = pl.multiple_of(j * CHUNK, CHUNK)
            kwin = kf_s[pl.ds(r0, CHUNK + 8), :]
            ks = kwin[8:, :] * taps[0:1, :]
            for t in range(1, n_taps):
                ks = ks + kwin[8 - t:8 - t + CHUNK, :] * taps[t:t + 1, :]
            kv = (ks * v_s[c, pl.ds(r0, CHUNK), :].astype(_F32)).astype(_BF16)
            b_s[c, pl.ds(r0, CHUNK), :] = kv.astype(_F32) * ssm_d
            xh_s[j] = jnp.dot(fwd, kv, preferred_element_type=_F32)
            kh_s[j] = lax.dot_general(
                fwd, ssmk_s[c, :, pl.ds(r0, CHUNK)], _NT, preferred_element_type=_F32)
            return carry

        lax.fori_loop(0, n_chunks, fwd_chunk, 0, unroll=4)

        def freq_group(g, carry):
            re = pl.ds(pl.multiple_of(g * 8, 8), 8)
            im = pl.ds(pl.multiple_of(CHUNK + g * 8, 8), 8)
            prev_r = prev_i = None
            blk = 4
            for i0 in range(0, n_chunks, blk):
                acc_r = [None] * blk
                acc_i = [None] * blk
                for j in range(i0 + blk):
                    xr, xi = xh_s[j, re, :], xh_s[j, im, :]
                    for b in range(blk):
                        d = i0 + b - j
                        if d < 0:
                            continue
                        kr, ki = kh_s[d, re, :], kh_s[d, im, :]
                        pr = xr * kr - xi * ki
                        pi = xr * ki + xi * kr
                        acc_r[b] = pr if acc_r[b] is None else acc_r[b] + pr
                        acc_i[b] = pi if acc_i[b] is None else acc_i[b] + pi
                for b in range(blk):
                    yr, yi = acc_r[b], acc_i[b]
                    if prev_r is not None:
                        yr, yi = yr - sign * prev_i, yi + sign * prev_r
                    yh_s[i0 + b, re, :] = yr
                    yh_s[i0 + b, im, :] = yi
                    prev_r, prev_i = acc_r[b], acc_i[b]
            return carry

        lax.fori_loop(0, CHUNK // 8, freq_group, 0)

        def inv_chunk(i, carry, c=c):
            r = pl.ds(pl.multiple_of(i * CHUNK, CHUNK), CHUNK)
            y = jnp.dot(inv, yh_s[i].astype(_BF16), preferred_element_type=_F32)
            b_s[c, r, :] = x_s[c, r, :].astype(_F32) * (y + b_s[c, r, :])
            return carry

        lax.fori_loop(0, n_chunks, inv_chunk, 0, unroll=4)

    tiles_per_chunk = n_wt // W_DMA_CHUNKS
    for j in range(W_DMA_CHUNKS):
        for m in range(3):
            w_copy(m, j).wait()

            def tr(t, carry, m=m, j=j):
                t = j * tiles_per_chunk + t
                r = pl.ds(pl.multiple_of(t * LANES, LANES), LANES)
                w_s[m, t] = wt_s[m, r, :].T
                return carry

            lax.fori_loop(0, tiles_per_chunk, tr, 0, unroll=2)
    for c in range(n_ct):
        wo_copy(c).wait()

    qi = lax.broadcasted_iota(jnp.int32, (rows, 2 * rows), 0)
    col = lax.broadcasted_iota(jnp.int32, (rows, 2 * rows), 1)
    head0 = col < rows
    kj = jnp.where(head0, col, col - rows)
    allowed = (qi >= seg) | (kj >= seg) | (qi >= kj)
    lane = lax.broadcasted_iota(jnp.int32, (rows, LANES), 1)
    low_half = lane < (d_head - LANES)
    zeros = jnp.zeros((rows, LANES), _F32)
    gate_w = gate_ref[...].astype(_F32)

    def project(h, m, p):
        return [
            jnp.dot(h, w_s[m, p * pair_t + t], preferred_element_type=_F32)
            for t in range(pair_t)
        ]

    def block_diag(t):
        top = jnp.concatenate([t[0], jnp.where(low_half, t[1], 0.0), zeros], axis=1)
        bot = jnp.concatenate([zeros, jnp.where(low_half, 0.0, t[1]), t[2]], axis=1)
        return jnp.concatenate([top, bot], axis=0).astype(_BF16)

    def softmax_pair(s):
        s = jnp.where(allowed, s * scale, -1e9)
        m0 = jnp.max(jnp.where(head0, s, -jnp.inf), axis=1, keepdims=True)
        m1 = jnp.max(jnp.where(head0, -jnp.inf, s), axis=1, keepdims=True)
        e = jnp.exp(s - jnp.where(head0, m0, m1))
        l0 = jnp.sum(jnp.where(head0, e, 0.0), axis=1, keepdims=True)
        l1 = jnp.sum(jnp.where(head0, 0.0, e), axis=1, keepdims=True)
        return e / jnp.where(head0, l0, l1)

    def out_copy(s):
        r = pl.ds(pl.multiple_of(s * seg, seg), seg)
        return pltpu.make_async_copy(out_s.at[r, :], out_hbm.at[r, :], out_sem)

    def step(s, mem):
        r = pl.ds(pl.multiple_of(s * seg, seg), seg)
        xs = jnp.concatenate([x_s[c, r, :] for c in range(n_ct)], axis=1).astype(_F32)
        h = jnp.concatenate([xs, mem], axis=0)
        q, kb, vb, prob, o = {}, {}, {}, {}, {}
        acc = [None] * n_ct
        for slot in range(n_pairs + LAG_O):
            p = slot
            if p < n_pairs:
                q[p] = jnp.concatenate(project(h, 0, p), axis=1)
                kb[p] = block_diag(project(h, 1, p))
                vb[p] = block_diag(project(h, 2, p))
            p = slot - LAG_S
            if 0 <= p < n_pairs:
                sc = lax.dot_general(q.pop(p), kb.pop(p), _NT, preferred_element_type=_F32)
                prob[p] = softmax_pair(sc)
            p = slot - LAG_PV
            if 0 <= p < n_pairs:
                o[p] = jnp.dot(prob.pop(p), vb.pop(p), preferred_element_type=_F32)
            p = slot - LAG_O
            if 0 <= p < n_pairs:
                op = o.pop(p)
                for c in range(n_ct):
                    y = jnp.dot(op, wo_s[c, p * pair_w:(p + 1) * pair_w, :],
                                preferred_element_type=_F32)
                    acc[c] = y if acc[c] is None else acc[c] + y
        a = jnp.concatenate(acc, axis=1)
        g = jax.nn.sigmoid(jnp.sum(xs * gate_w, axis=1, keepdims=True))
        b = jnp.concatenate([b_s[c, r, :] for c in range(n_ct)], axis=1)
        out_s[r, :] = (g * a[:seg] + (1.0 - g) * b).astype(out_s.dtype)
        out_copy(s).start()
        return a[seg:]

    lax.fori_loop(0, n_seg, step, mem0_ref[...].astype(_F32))
    pltpu.make_async_copy(out_s, out_hbm, out_sem).wait()


@functools.partial(jax.jit, static_argnames=("A_seg_len",))
def pallas_gated_mix__memory_aug_recurrent_mem_tr__ssm_conv_h3__prompt_kernel(
    A_x: jax.Array,
    A_mem0: jax.Array,
    A_Wq: jax.Array,
    A_Wk: jax.Array,
    A_Wv: jax.Array,
    A_Wo: jax.Array,
    A_seg_len: int,
    B_q: jax.Array,
    B_k: jax.Array,
    B_v: jax.Array,
    B_shift_k: jax.Array,
    B_ssm_k: jax.Array,
    B_ssm_D: jax.Array,
    gate_w: jax.Array,
):
    del B_q
    batch, seq, d_model = A_x.shape
    n_mem = A_mem0.shape[1]
    _, n_heads, d_head = A_Wq.shape
    seg = int(A_seg_len)
    inner = n_heads * d_head
    n_ct = d_model // LANES
    n_chunks = seq // CHUNK
    assert batch == 1 and d_model % LANES == 0 and seq % (4 * CHUNK) == 0
    assert seq % seg == 0 and seg % 16 == 0 and n_mem % 8 == 0
    assert n_heads % 2 == 0 and 2 * d_head == 3 * LANES and 2 * (seg + n_mem) <= LANES

    def feature_major(w):
        return jnp.transpose(w, (1, 2, 0)).reshape(inner, d_model)

    fwd, inv = _dft_constants()
    any_spec = pl.BlockSpec(memory_space=pl.ANY)
    vmem_spec = pl.BlockSpec(memory_space=pltpu.VMEM)
    out = pl.pallas_call(
        functools.partial(_kernel, seg=seg, n_mem=n_mem, n_heads=n_heads, d_head=d_head),
        out_shape=jax.ShapeDtypeStruct((seq, d_model), A_x.dtype),
        in_specs=[
            any_spec, vmem_spec, any_spec, any_spec, any_spec, any_spec, any_spec,
            any_spec, vmem_spec, any_spec, vmem_spec, vmem_spec, vmem_spec, vmem_spec,
        ],
        out_specs=any_spec,
        scratch_shapes=[
            pltpu.VMEM((n_ct, seq, LANES), _BF16),
            pltpu.VMEM((n_ct, seq, LANES), _BF16),
            pltpu.VMEM((n_ct, seq, LANES), _BF16),
            pltpu.VMEM((n_ct, LANES, seq), _BF16),
            pltpu.VMEM((3, inner, d_model), _BF16),
            pltpu.VMEM((3, inner // LANES, d_model, LANES), _BF16),
            pltpu.VMEM((n_ct, inner, LANES), _BF16),
            pltpu.VMEM((seq + 8, LANES), _F32),
            pltpu.VMEM((n_chunks, 2 * CHUNK, LANES), _F32),
            pltpu.VMEM((n_chunks, 2 * CHUNK, LANES), _F32),
            pltpu.VMEM((n_chunks, 2 * CHUNK, LANES), _F32),
            pltpu.VMEM((n_ct, seq, LANES), _F32),
            pltpu.VMEM((seq, d_model), A_x.dtype),
            pltpu.SemaphoreType.DMA((4, n_ct)),
            pltpu.SemaphoreType.DMA((3, W_DMA_CHUNKS)),
            pltpu.SemaphoreType.DMA((n_ct,)),
            pltpu.SemaphoreType.DMA(()),
        ],
        compiler_params=pltpu.CompilerParams(vmem_limit_bytes=110 * 1024 * 1024),
        name="gated_mix_rmt_h3",
    )(
        A_x.reshape(seq, d_model),
        A_mem0.reshape(n_mem, d_model),
        feature_major(A_Wq),
        feature_major(A_Wk),
        feature_major(A_Wv),
        A_Wo.reshape(inner, d_model),
        B_k.reshape(seq, d_model),
        B_v.reshape(seq, d_model),
        B_shift_k.T,
        B_ssm_k,
        B_ssm_D.reshape(1, d_model),
        gate_w.reshape(1, d_model),
        jnp.asarray(fwd, _BF16),
        jnp.asarray(inv, _BF16),
    )
    return out.reshape(batch, seq, d_model)
```

```python
import functools

import jax
import jax.numpy as jnp
import numpy as np
from jax import lax
import jax.experimental.pallas as pl
import jax.experimental.pallas.tpu as pltpu

LANES = 128
CHUNK = 128
UNROLL = 3
NIT_DBG = None
PROD_UNROLL = 4

LAG_S, LAG_PV, LAG_O = 1, 3, 5

_F32 = jnp.float32
_BF16 = jnp.bfloat16
_NT = (((1,), (1,)), ((), ()))


def _dft_constants():
    w = np.pi * (np.arange(CHUNK, dtype=np.float64) + 0.5) / CHUNK
    t = np.arange(CHUNK, dtype=np.float64)
    ang = w[:, None] * t[None, :]
    fwd = np.concatenate([np.cos(ang), -np.sin(ang)], axis=0)
    inv = np.concatenate([np.cos(ang.T), -np.sin(ang.T)], axis=1) / CHUNK
    return fwd.astype(np.float32), inv.astype(np.float32)


def _dot(a, b):
    return jnp.dot(a, b, preferred_element_type=_F32)


def _kernel(
    x_hbm, mem0_ref, wq_hbm, wk_hbm, wv_hbm, wo_hbm, k_hbm, v_hbm,
    shift_ref, ssmk_hbm, ssmd_ref, gate_ref, fwd_ref, inv_ref,
    out_hbm,
    x_s, k_s, v_s, ssmk_s, wt_s, w_s, wo_s, kf_s, xh_s, kh_s, yh_s,
    b_s, out_s, in_sem, w_sem, x_sem, out_sem,
    *, seg, n_mem, n_heads, d_head,
):
    n_ct, seq, _ = k_s.shape
    n_chunks = seq // CHUNK
    n_seg = seq // seg
    rows = seg + n_mem
    n_pairs = n_heads // 2
    pair_w = 2 * d_head
    pair_t = pair_w // LANES
    scale = float(d_head) ** -0.5
    n_taps = shift_ref.shape[0]
    x_head = (1 + UNROLL) * seg

    def act_copies(c):
        cols = pl.ds(pl.multiple_of(c * LANES, LANES), LANES)
        return (
            pltpu.make_async_copy(k_hbm.at[:, cols], k_s.at[c], in_sem.at[0, c]),
            pltpu.make_async_copy(v_hbm.at[:, cols], v_s.at[c], in_sem.at[1, c]),
            pltpu.make_async_copy(ssmk_hbm.at[cols, :], ssmk_s.at[c], in_sem.at[2, c]),
        )

    def w_copy(m, p):
        src = (wq_hbm, wk_hbm, wv_hbm, wo_hbm)[m]
        r = pl.ds(pl.multiple_of(p * pair_w, pair_w), pair_w)
        return pltpu.make_async_copy(src.at[r, :], wt_s.at[m, r, :], w_sem.at[m, p])

    def x_copy(j):
        r = pl.ds(0, x_head) if j == 0 else pl.ds(x_head, seq - x_head)
        return pltpu.make_async_copy(x_hbm.at[r, :], x_s.at[r, :], x_sem.at[j])

    @pl.loop(0, n_ct)
    def _(c):
        for cp in act_copies(c):
            cp.start()

    x_copy(0).start()

    def start_weights(lo, hi):
        @pl.loop(lo, hi)
        def _(p):
            for m in range(4):
                w_copy(m, p).start()

    batch = (0, 3 * n_pairs // 8, 11 * n_pairs // 16, n_pairs)
    start_weights(batch[0], batch[1])

    kf_s[0:8, :] = jnp.zeros((8, LANES), _F32)
    sub = lax.broadcasted_iota(jnp.int32, (CHUNK, LANES), 0)
    sign = jnp.where(sub % 2 == 0, 1.0, -1.0).astype(_F32)

    def forward(c, j):
        cols = slice(c * LANES, (c + 1) * LANES)
        taps = shift_ref[:, cols].astype(_F32)
        r0 = j * CHUNK
        ks = kf_s[pl.ds(r0 + 8, CHUNK), :] * taps[0:1, :]
        for t in range(1, n_taps):
            ks = ks + kf_s[pl.ds(r0 + 8 - t, CHUNK), :] * taps[t:t + 1, :]
        kv = (ks * v_s[c, pl.ds(r0, CHUNK), :].astype(_F32)).astype(_BF16)
        b_s[c, pl.ds(r0, CHUNK), :] = kv.astype(_F32) * ssmd_ref[:, cols].astype(_F32)
        xf = _dot(fwd_ref[...], kv)
        xr, xi = xf[:CHUNK], xf[CHUNK:]
        xh_s[j] = jnp.concatenate([xr + xi, xr, xi], axis=0)
        kf = lax.dot_general(fwd_ref[...], ssmk_s[c, :, pl.ds(r0, CHUNK)], _NT,
                             preferred_element_type=_F32)
        kr, ki = kf[:CHUNK], kf[CHUNK:]
        kh_s[j] = jnp.concatenate([kr, ki - kr, kr + ki], axis=0)

    def product_sum(g, carry):
        f = pl.ds(pl.multiple_of(g * 8, 8), 8)
        xs, ks = [], []
        for i in range(n_chunks):
            xs.append(xh_s[i, f, :])
            ks.append(kh_s[i, f, :])
            acc = xs[0] * ks[i]
            for j in range(1, i + 1):
                acc = acc + xs[j] * ks[i - j]
            yh_s[i, f, :] = acc
        return carry

    def spectrum(i):
        a0, a1, a2 = (yh_s[i, n * CHUNK:(n + 1) * CHUNK, :] for n in range(3))
        return a0 - a2, a0 + a1

    def inverse(c, i):
        yr, yi = spectrum(i)
        if i > 0:
            pr, pi = spectrum(i - 1)
            yr, yi = yr - sign * pi, yi + sign * pr
        yf = jnp.concatenate([yr, yi], axis=0).astype(_BF16)
        b_s[c, pl.ds(i * CHUNK, CHUNK), :] += _dot(inv_ref[...], yf)

    for c in range(n_ct + 1):
        if c < n_ct:
            with jax.named_scope(f"wait{c}"):
                for cp in act_copies(c):
                    cp.wait()
            kf_s[8:, :] = k_s[c].astype(_F32)
        with jax.named_scope(f"dft{c}"):
            for j in range(n_chunks):
                if c < n_ct:
                    forward(c, j)
                if c > 0:
                    inverse(c - 1, j)
        if c < n_ct:
            with jax.named_scope(f"prod{c}"):
                lax.fori_loop(0, 3 * CHUNK // 8, product_sum, 0, unroll=PROD_UNROLL)
        if c == 1:
            start_weights(batch[1], batch[2])
        if c == n_ct - 1:
            start_weights(batch[2], batch[3])
            x_copy(1).start()

    qi = lax.broadcasted_iota(jnp.int32, (rows, 2 * rows), 0)
    col = lax.broadcasted_iota(jnp.int32, (rows, 2 * rows), 1)
    head0 = col < rows
    kj = jnp.where(head0, col, col - rows)
    allowed = (qi >= seg) | (kj >= seg) | (qi >= kj)
    lane = lax.broadcasted_iota(jnp.int32, (rows, LANES), 1)
    low_half = lane < (d_head - LANES)
    zeros = jnp.zeros((rows, LANES), _F32)
    gate_w = gate_ref[...].astype(_F32)

    def project(h, m, p):
        return [
            _dot(h, pltpu.bitcast(w_s[m, p * pair_t + t], _BF16))
            for t in range(pair_t)
        ]

    def block_diag(t):
        top = jnp.concatenate([t[0], jnp.where(low_half, t[1], 0.0), zeros], axis=1)
        bot = jnp.concatenate([zeros, jnp.where(low_half, 0.0, t[1]), t[2]], axis=1)
        return jnp.concatenate([top, bot], axis=0).astype(_BF16)

    def qkv(h, p, project=project):
        return (jnp.concatenate(project(h, 0, p), axis=1),
                block_diag(project(h, 1, p)), block_diag(project(h, 2, p)))

    def probabilities(q, kb):
        s = lax.dot_general(q, kb, _NT, preferred_element_type=_F32)
        s = jnp.where(allowed, s * scale, -1e9)
        m0 = jnp.max(jnp.where(head0, s, -jnp.inf), axis=1, keepdims=True)
        m1 = jnp.max(jnp.where(head0, -jnp.inf, s), axis=1, keepdims=True)
        e = jnp.exp(s - jnp.where(head0, m0, m1))
        l0 = jnp.sum(jnp.where(head0, e, 0.0), axis=1, keepdims=True)
        l1 = jnp.sum(jnp.where(head0, 0.0, e), axis=1, keepdims=True)
        return e / jnp.where(head0, l0, l1)

    def out_project(o, p):
        o = jnp.concatenate([o[seg:], o[:seg]], axis=0)
        ys = []
        for c in range(n_ct):
            w = jnp.concatenate(
                [wo_s[p * pair_t + t, :, c * LANES:(c + 1) * LANES]
                 for t in range(pair_t)], axis=0)
            ys.append(_dot(o, pltpu.bitcast(w, _BF16)))
        return ys

    def seg_rows(s):
        return pl.ds(pl.multiple_of(s * seg, seg), seg)

    def finish(s, xs, acc):
        a = jnp.concatenate(acc, axis=1)
        g = jax.nn.sigmoid(jnp.sum(xs * gate_w, axis=1, keepdims=True))
        b = xs * jnp.concatenate([b_s[c, seg_rows(s), :] for c in range(n_ct)], axis=1)
        out_s[seg_rows(s), :] = (g * a[n_mem:] + (1.0 - g) * b).astype(out_s.dtype)
        return a[:n_mem]

    x_copy(0).wait()
    xs0 = x_s[0:seg, :].astype(_F32)
    h0 = jnp.concatenate([xs0, mem0_ref[...].astype(_F32)], axis=0)

    def staged(m, p, t):
        return wt_s[m, pl.ds(pl.multiple_of((p * pair_t + t) * LANES, LANES), LANES), :]

    def project_staged(h, m, p):
        return [lax.dot_general(h, staged(m, p, t), _NT, preferred_element_type=_F32)
                for t in range(pair_t)]

    def first_step(p, acc):
        with jax.named_scope("wwait"):
            for m in range(4):
                w_copy(m, p).wait()
        for m in range(3):
            for t in range(pair_t):
                w_s[m, p * pair_t + t] = pltpu.bitcast(staged(m, p, t).T, jnp.int32)
        q, kb, vb = qkv(h0, p, project_staged)
        o = _dot(probabilities(q, kb), vb)
        for t in range(pair_t):
            wo_s[p * pair_t + t] = pltpu.bitcast(staged(3, p, t), jnp.int32)
        return [a + y for a, y in zip(acc, out_project(o, p))]

    with jax.named_scope("first"):
        acc0 = lax.fori_loop(0, n_pairs, first_step, [zeros] * n_ct)
    mem1 = finish(0, xs0, acc0)

    def step(s, mem):
        xs = x_s[seg_rows(s), :].astype(_F32)
        h = jnp.concatenate([xs, mem], axis=0)
        q, kb, vb, prob, o = {}, {}, {}, {}, {}
        acc = None
        for slot in range(n_pairs + LAG_O):
            p = slot
            if p < n_pairs:
                q[p], kb[p], vb[p] = qkv(h, p)
            p = slot - LAG_S
            if 0 <= p < n_pairs:
                prob[p] = probabilities(q.pop(p), kb.pop(p))
            p = slot - LAG_PV
            if 0 <= p < n_pairs:
                o[p] = _dot(prob.pop(p), vb.pop(p))
            p = slot - LAG_O
            if 0 <= p < n_pairs:
                ys = out_project(o.pop(p), p)
                acc = ys if acc is None else [a + y for a, y in zip(acc, ys)]
        return finish(s, xs, acc)

    def out_copy(start, size):
        r = pl.ds(pl.multiple_of(start, seg), size)
        return pltpu.make_async_copy(out_s.at[r, :], out_hbm.at[r, :], out_sem)

    def steps(i, mem):
        @pl.when(i == 1)
        def _():
            x_copy(1).wait()

        @pl.when(i > 0)
        def _():
            out_copy((1 + (i - 1) * UNROLL) * seg, UNROLL * seg).start()

        for u in range(UNROLL):
            mem = step(1 + i * UNROLL + u, mem)
        return mem

    out_copy(0, seg).start()
    n_it = (n_seg - 1) // UNROLL if NIT_DBG is None else NIT_DBG
    with jax.named_scope("main"):
        lax.fori_loop(0, n_it, steps, mem1)
    out_copy((1 + (n_it - 1) * UNROLL) * seg, UNROLL * seg).start()
    out_copy(0, (1 + n_it * UNROLL) * seg).wait()


@functools.partial(jax.jit, static_argnames=("A_seg_len",))
def pallas_gated_mix__memory_aug_recurrent_mem_tr__ssm_conv_h3__prompt_kernel(
    A_x: jax.Array,
    A_mem0: jax.Array,
    A_Wq: jax.Array,
    A_Wk: jax.Array,
    A_Wv: jax.Array,
    A_Wo: jax.Array,
    A_seg_len: int,
    B_q: jax.Array,
    B_k: jax.Array,
    B_v: jax.Array,
    B_shift_k: jax.Array,
    B_ssm_k: jax.Array,
    B_ssm_D: jax.Array,
    gate_w: jax.Array,
):
    del B_q
    batch, seq, d_model = A_x.shape
    n_mem = A_mem0.shape[1]
    _, n_heads, d_head = A_Wq.shape
    seg = int(A_seg_len)
    inner = n_heads * d_head
    n_ct = d_model // LANES
    n_chunks = seq // CHUNK
    assert batch == 1 and d_model % LANES == 0 and n_chunks * 8 == CHUNK
    assert seq % seg == 0 and seg % 16 == 0 and n_mem % 8 == 0
    assert (seq // seg - 1) % UNROLL == 0 and seq // seg > 1 + UNROLL
    assert n_heads % 2 == 0 and 2 * d_head == 3 * LANES and 2 * (seg + n_mem) <= LANES

    def feature_major(w):
        return jnp.transpose(w, (1, 2, 0)).reshape(inner, d_model)

    fwd, inv = _dft_constants()
    any_spec = pl.BlockSpec(memory_space=pl.ANY)
    vmem_spec = pl.BlockSpec(memory_space=pltpu.VMEM)
    out = pl.pallas_call(
        functools.partial(_kernel, seg=seg, n_mem=n_mem, n_heads=n_heads, d_head=d_head),
        out_shape=jax.ShapeDtypeStruct((seq, d_model), A_x.dtype),
        in_specs=[
            any_spec, vmem_spec, any_spec, any_spec, any_spec, any_spec, any_spec,
            any_spec, vmem_spec, any_spec, vmem_spec, vmem_spec, vmem_spec, vmem_spec,
        ],
        out_specs=any_spec,
        scratch_shapes=[
            pltpu.VMEM((seq, d_model), _BF16),
            pltpu.VMEM((n_ct, seq, LANES), _BF16),
            pltpu.VMEM((n_ct, seq, LANES), _BF16),
            pltpu.VMEM((n_ct, LANES, seq), _BF16),
            pltpu.VMEM((4, inner, d_model), _BF16),
            pltpu.VMEM((3, inner // LANES, d_model // 2, LANES), jnp.int32),
            pltpu.VMEM((inner // LANES, LANES // 2, d_model), jnp.int32),
            pltpu.VMEM((seq + 8, LANES), _F32),
            pltpu.VMEM((n_chunks, 3 * CHUNK, LANES), _F32),
            pltpu.VMEM((n_chunks, 3 * CHUNK, LANES), _F32),
            pltpu.VMEM((n_chunks, 3 * CHUNK, LANES), _F32),
            pltpu.VMEM((n_ct, seq, LANES), _F32),
            pltpu.VMEM((seq, d_model), A_x.dtype),
            pltpu.SemaphoreType.DMA((3, n_ct)),
            pltpu.SemaphoreType.DMA((4, n_heads // 2)),
            pltpu.SemaphoreType.DMA((2,)),
            pltpu.SemaphoreType.DMA(()),
        ],
        compiler_params=pltpu.CompilerParams(vmem_limit_bytes=112 * 1024 * 1024),
        name="gated_mix_rmt_h3",
    )(
        A_x.reshape(seq, d_model),
        A_mem0.reshape(n_mem, d_model),
        feature_major(A_Wq),
        feature_major(A_Wk),
        feature_major(A_Wv),
        A_Wo.reshape(inner, d_model),
        B_k.reshape(seq, d_model),
        B_v.reshape(seq, d_model),
        B_shift_k.T,
        B_ssm_k,
        B_ssm_D.reshape(1, d_model),
        gate_w.reshape(1, d_model),
        jnp.asarray(fwd, _BF16),
        jnp.asarray(inv, _BF16),
    )
    return out.reshape(batch, seq, d_model)
```

```python
import functools

import jax
import jax.numpy as jnp
import numpy as np
from jax import lax
import jax.experimental.pallas as pl
import jax.experimental.pallas.tpu as pltpu

LANES = 128
CHUNK = 128
PLANES = 3
LATE = 3
UNROLL = 3
PRE = 8
N_PRE = 33
CONV_UNROLL = 4
TIE = 3

LAG_S, LAG_PV, LAG_O = 1, 4, 6

_F32 = jnp.float32
_BF16 = jnp.bfloat16
_NT = (((1,), (1,)), ((), ()))


def _dft_constants():
    w = np.pi * (np.arange(CHUNK, dtype=np.float64) + 0.5) / CHUNK
    t = np.arange(CHUNK, dtype=np.float64)
    ang = w[:, None] * t[None, :]
    fwd = np.concatenate([np.cos(ang), -np.sin(ang)], axis=0)
    inv = np.concatenate([np.cos(ang.T), -np.sin(ang.T)], axis=1) / CHUNK
    return fwd.astype(np.float32), inv.astype(np.float32)


def _dot(a, b):
    return jnp.dot(a, b, preferred_element_type=_F32)


def _dot_nt(a, b):
    return lax.dot_general(a, b, _NT, preferred_element_type=_F32)


def _rows(start, size, align):
    return pl.ds(start if isinstance(start, int) else pl.multiple_of(start, align), size)


def _kernel(
    x_hbm, wq_hbm, wk_hbm, wv_hbm, wo_hbm, k_hbm, v_hbm, ssmk_hbm,
    mem0_hbm, taps_hbm, ssmd_hbm, gate_hbm, fwd_hbm, inv_hbm,
    out_hbm,
    mem0_s, taps_s, ssmd_s, gate_s, fwd_s, inv_s,
    x_s, k_s, v_s, ssmk_s, wt_s, w_s, wo_s, kf_s, xh_s, kh_s, b_s, pre_s, h0_s, out_s, ones_s,
    small_sem, in_sem, w_sem, x_sem, out_sem,
    *, seg, n_heads, d_head,
):
    n_ct, seq, _ = k_s.shape
    d_model = n_ct * LANES
    n_mem = mem0_s.shape[0]
    n_taps = taps_s.shape[0]
    n_chunks = seq // CHUNK
    n_seg = seq // seg
    rows = seg + n_mem
    n_pairs = n_heads // 2
    pair_w = 2 * d_head
    pair_t = pair_w // LANES
    scale = float(d_head) ** -0.5
    x_head = (1 + N_PRE) * seg
    spec = PLANES * CHUNK

    small_copies = [
        pltpu.make_async_copy(src, dst, small_sem.at[i])
        for i, (src, dst) in enumerate((
            (fwd_hbm, fwd_s), (taps_hbm, taps_s), (ssmd_hbm, ssmd_s),
            (inv_hbm, inv_s), (mem0_hbm, mem0_s), (gate_hbm, gate_s)))
    ]

    def act_copies(c):
        cols = _rows(c * LANES, LANES, LANES)
        return (
            pltpu.make_async_copy(ssmk_hbm.at[cols, :], ssmk_s.at[c], in_sem.at[0, c]),
            pltpu.make_async_copy(k_hbm.at[:, cols], k_s.at[c], in_sem.at[1, c]),
            pltpu.make_async_copy(v_hbm.at[:, cols], v_s.at[c], in_sem.at[2, c]),
        )

    def w_copy(m, p):
        src = (wq_hbm, wk_hbm, wv_hbm, wo_hbm)[m]
        r = _rows(p * pair_w, pair_w, pair_w)
        return pltpu.make_async_copy(src.at[r, :], wt_s.at[m, r, :], w_sem.at[m, p])

    def x_copy(j):
        r = pl.ds(0, x_head) if j == 0 else pl.ds(x_head, seq - x_head)
        return pltpu.make_async_copy(x_hbm.at[r, :], x_s.at[r, :], x_sem.at[j])

    def start_weights(lo, hi):
        @pl.loop(lo, hi)
        def _(p):
            for m in range(4):
                w_copy(m, p).start()

    for cp in small_copies:
        cp.start()

    @pl.loop(0, n_ct)
    def _(c):
        for cp in act_copies(c):
            cp.start()

    x_copy(0).start()
    batch = (0, 5 * n_pairs // 16, 9 * n_pairs // 16, n_pairs)
    start_weights(batch[0], batch[1])
    for cp in small_copies:
        cp.wait()

    kf_s[0:8, :] = jnp.zeros((8, LANES), _F32)
    freq = lax.broadcasted_iota(jnp.int32, (CHUNK, LANES), 0)
    sign = jnp.where(freq % 2 == 0, 1.0, -1.0).astype(_F32)
    ssm_d = ssmd_s[...].astype(_F32).reshape(1, d_model)

    def slot(c):
        return pl.ds((c % LATE) * spec, spec)

    def filter_spectrum(c, j):
        kf = _dot_nt(fwd_s[...], ssmk_s[c, :, j * CHUNK:(j + 1) * CHUNK])
        kr, ki = kf[:CHUNK], kf[CHUNK:]
        kh_s[j, slot(c), :] = jnp.concatenate([kr, ki - kr, kr + ki], axis=0)

    def signal_spectrum(c, j):
        cols = slice(c * LANES, (c + 1) * LANES)
        taps = taps_s[:, cols].astype(_F32)
        r0 = j * CHUNK
        ks = kf_s[pl.ds(r0 + 8, CHUNK), :] * taps[0:1, :]
        for t in range(1, n_taps):
            ks = ks + kf_s[pl.ds(r0 + 8 - t, CHUNK), :] * taps[t:t + 1, :]
        kv = (ks * v_s[c, pl.ds(r0, CHUNK), :].astype(_F32)).astype(_BF16)
        b_s[c, pl.ds(r0, CHUNK), :] = kv.astype(_F32) * ssm_d[:, cols]
        xf = _dot(fwd_s[...], kv)
        xr, xi = xf[:CHUNK], xf[CHUNK:]
        xh_s[j, slot(c), :] = jnp.concatenate([xr + xi, xr, xi], axis=0)

    def tie(value, other):
        return jnp.where(ones_s[...] > 0, value, other)

    def chunk_conv(g, after=None):
        f = _rows(g * 8, 8, 8)
        xs, ks = [], []
        for i in range(n_chunks):
            xs.append(xh_s[i, f, :])
            if i == 0 and after is not None:
                xs[0] = tie(xs[0], after)
            ks.append(kh_s[i, f, :])
            acc = xs[0] * ks[i]
            for j in range(1, i + 1):
                acc = acc + xs[j] * ks[i - j]
            xh_s[i, f, :] = acc
        return acc

    def response(c, i):
        a = xh_s[i, slot(c), :]
        a0, a1, a2 = (a[n * CHUNK:(n + 1) * CHUNK] for n in range(PLANES))
        return a0 - a2, a0 + a1

    def inverse(c, i):
        yr, yi = response(c, i)
        if i > 0:
            pr, pi = response(c, i - 1)
            yr, yi = yr - sign * pi, yi + sign * pr
        yf = jnp.concatenate([yr, yi], axis=0).astype(_BF16)
        b_s[c, i * CHUNK:(i + 1) * CHUNK, :] += _dot(inv_s[...], yf)

    n_early = n_ct - LATE
    for c in range(n_ct):
        filt, key, val = act_copies(c)
        filt.wait()
        if c == 0:
            for j in range(n_chunks):
                filter_spectrum(c, j)
        key.wait()
        val.wait()
        kf_s[8:, :] = k_s[c].astype(_F32)
        for j in range(n_chunks):
            signal_spectrum(c, j)
            if c > 0:
                filter_spectrum(c, j)
            if 0 < c <= n_early:
                inverse(c - 1, j)
        if c < n_early:
            g0 = (c % LATE) * spec // 8

            @pl.loop(g0, g0 + spec // 8, unroll=CONV_UNROLL)
            def _(g):
                chunk_conv(g)

        if c == 1:
            start_weights(batch[1], batch[2])
    start_weights(batch[2], batch[3])
    x_copy(1).start()

    qi = lax.broadcasted_iota(jnp.int32, (rows, 2 * rows), 0)
    col = lax.broadcasted_iota(jnp.int32, (rows, 2 * rows), 1)
    head0 = col < rows
    kj = jnp.where(head0, col, col - rows)
    allowed = (qi >= seg) | (kj >= seg) | (qi >= kj)
    lane = lax.broadcasted_iota(jnp.int32, (rows, LANES), 1)
    low_half = lane < (d_head - LANES)
    zeros = jnp.zeros((rows, LANES), _F32)
    gate_w = gate_s[...].astype(_F32).reshape(1, d_model)

    def block_diag(t):
        top = jnp.concatenate([t[0], jnp.where(low_half, t[1], 0.0), zeros], axis=1)
        bot = jnp.concatenate([zeros, jnp.where(low_half, 0.0, t[1]), t[2]], axis=1)
        return jnp.concatenate([top, bot], axis=0).astype(_BF16)

    def probabilities(q, kb):
        s = jnp.where(allowed, _dot_nt(q, kb) * scale, -1e9)
        m0 = jnp.max(jnp.where(head0, s, -jnp.inf), axis=1, keepdims=True)
        m1 = jnp.max(jnp.where(head0, -jnp.inf, s), axis=1, keepdims=True)
        e = jnp.exp(s - jnp.where(head0, m0, m1))
        l0 = jnp.sum(jnp.where(head0, e, 0.0), axis=1, keepdims=True)
        l1 = jnp.sum(jnp.where(head0, 0.0, e), axis=1, keepdims=True)
        return e / jnp.where(head0, l0, l1)

    def out_project(o, p):
        o = jnp.concatenate([o[seg:], o[:seg]], axis=0)
        ys = []
        for c in range(n_ct):
            w = jnp.concatenate(
                [wo_s[p * pair_t + t, :, c * LANES:(c + 1) * LANES]
                 for t in range(pair_t)], axis=0)
            ys.append(_dot(o, pltpu.bitcast(w, _BF16)))
        return ys

    def add(acc, ys):
        return [a + y for a, y in zip(acc, ys)]

    def finish(s, xs, acc):
        r = _rows(s * seg, seg, seg)
        a = jnp.concatenate(acc, axis=1)
        g = jax.nn.sigmoid(jnp.sum(xs * gate_w, axis=1, keepdims=True))
        b = xs * jnp.concatenate([b_s[c, r, :] for c in range(n_ct)], axis=1)
        out_s[r, :] = (g * a[n_mem:] + (1.0 - g) * b).astype(out_s.dtype)
        return a[:n_mem]

    x_copy(0).wait()
    xs0 = x_s[0:seg, :].astype(_F32)
    h0_s[...] = pltpu.bitcast(jnp.concatenate(
        [xs0, mem0_s[...].astype(_F32)]
        + [x_s[s * seg:(s + 1) * seg, :].astype(_F32)[seg - PRE:]
           for s in range(1, 1 + N_PRE)], axis=0).astype(_BF16), jnp.int32)

    def staged(m, p, t):
        return wt_s[m, _rows((p * pair_t + t) * LANES, LANES, LANES), :]

    def project_staged(m, p, link):
        ys = []
        for t in range(pair_t):
            w = staged(m, p, t)
            w_s[m, p * pair_t + t] = pltpu.bitcast(w.T, jnp.int32)
            h = h0_s[...]
            if len(link) >= TIE:
                corner = tie(h[:8, :LANES], pltpu.bitcast(link[-TIE], jnp.int32))
                top = jnp.concatenate([corner, h[:8, LANES:]], axis=1)
                h = jnp.concatenate([top, h[8:]], axis=0)
            y = _dot_nt(pltpu.bitcast(h, _BF16), w)
            link.append(chunk_conv((p * 3 + m) * pair_t + t, y[:8]))
            pre_s[m, p * pair_t + t] = y[rows:]
            ys.append(y[:rows])
        return ys

    def repack_wo(p):
        for t in range(pair_t):
            wo_s[p * pair_t + t] = pltpu.bitcast(staged(3, p, t), jnp.int32)

    for m in range(3):
        w_copy(m, 0).wait()
    ones_s[...] = jnp.ones(ones_s.shape, jnp.int32)
    link = []
    first = (jnp.concatenate(project_staged(0, 0, link), axis=1),
             block_diag(project_staged(1, 0, link)), block_diag(project_staged(2, 0, link)))

    def first_step(p, carry):
        (q, kb, vb), acc = carry
        w_copy(3, p - 1).wait()
        for m in range(3):
            w_copy(m, p).wait()
        repack_wo(p - 1)
        prob = probabilities(q, kb)
        link = []
        q = jnp.concatenate(project_staged(0, p, link), axis=1)
        o = _dot(prob, vb)
        kb = block_diag(project_staged(1, p, link))
        acc = add(acc, out_project(o, p - 1))
        vb = block_diag(project_staged(2, p, link))
        return (q, kb, vb), acc

    (q, kb, vb), acc0 = lax.fori_loop(1, n_pairs, first_step, (first, [zeros] * n_ct))
    o = _dot(probabilities(q, kb), vb)
    for c in range(n_early, n_ct):
        for i in range(n_chunks):
            inverse(c, i)
    w_copy(3, n_pairs - 1).wait()
    repack_wo(n_pairs - 1)
    mem1 = finish(0, xs0, add(acc0, out_project(o, n_pairs - 1)))

    def project(h, m, p):
        return [_dot(h, pltpu.bitcast(w_s[m, p * pair_t + t], _BF16))
                for t in range(pair_t)]

    def project_rest(s, h, m, p):
        r = _rows((s - 1) * PRE, PRE, PRE)
        return [
            jnp.concatenate(
                [y[:seg - PRE], pre_s[m, p * pair_t + t, r, :], y[seg - PRE:]], axis=0)
            for t, y in enumerate(project(h, m, p))
        ]

    def step(s, mem, has_pre):
        xs = x_s[_rows(s * seg, seg, seg), :].astype(_F32)
        if has_pre:
            h = jnp.concatenate([xs[:seg - PRE], mem], axis=0).astype(_BF16)
            proj = functools.partial(project_rest, s)
        else:
            h = jnp.concatenate([xs, mem], axis=0)
            proj = project
        q, kb, vb, prob, o = {}, {}, {}, {}, {}
        acc = None
        for p in range(n_pairs + LAG_O):
            if p < n_pairs:
                q[p] = jnp.concatenate(proj(h, 0, p), axis=1)
                kb[p] = block_diag(proj(h, 1, p))
                vb[p] = block_diag(proj(h, 2, p))
            if 0 <= p - LAG_S < n_pairs:
                prob[p - LAG_S] = probabilities(q.pop(p - LAG_S), kb.pop(p - LAG_S))
            if 0 <= p - LAG_PV < n_pairs:
                o[p - LAG_PV] = _dot(prob.pop(p - LAG_PV), vb.pop(p - LAG_PV))
            if 0 <= p - LAG_O:
                ys = out_project(o.pop(p - LAG_O), p - LAG_O)
                acc = ys if acc is None else add(acc, ys)
        return finish(s, xs, acc)

    def out_copy(start, size):
        r = _rows(start, size, seg)
        return pltpu.make_async_copy(out_s.at[r, :], out_hbm.at[r, :], out_sem)

    def run(s0, n, has_pre, mem):
        def body(i, mem):
            @pl.when(i > 0)
            def _():
                out_copy((s0 + (i - 1) * UNROLL) * seg, UNROLL * seg).start()

            for u in range(UNROLL):
                mem = step(s0 + i * UNROLL + u, mem, has_pre)
            return mem

        mem = lax.fori_loop(0, n // UNROLL, body, mem)
        out_copy((s0 + n - UNROLL) * seg, UNROLL * seg).start()
        return mem

    out_copy(0, seg).start()
    mem = run(1, N_PRE, True, mem1)
    x_copy(1).wait()
    run(1 + N_PRE, n_seg - 1 - N_PRE, False, mem)
    out_copy(0, seq).wait()


@functools.partial(jax.jit, static_argnames=("A_seg_len",))
def pallas_gated_mix__memory_aug_recurrent_mem_tr__ssm_conv_h3__prompt_kernel(
    A_x: jax.Array,
    A_mem0: jax.Array,
    A_Wq: jax.Array,
    A_Wk: jax.Array,
    A_Wv: jax.Array,
    A_Wo: jax.Array,
    A_seg_len: int,
    B_q: jax.Array,
    B_k: jax.Array,
    B_v: jax.Array,
    B_shift_k: jax.Array,
    B_ssm_k: jax.Array,
    B_ssm_D: jax.Array,
    gate_w: jax.Array,
):
    del B_q
    batch, seq, d_model = A_x.shape
    n_mem = A_mem0.shape[1]
    _, n_heads, d_head = A_Wq.shape
    seg = int(A_seg_len)
    inner = n_heads * d_head
    n_ct = d_model // LANES
    n_chunks = seq // CHUNK
    assert batch == 1 and d_model % LANES == 0 and seq % CHUNK == 0 and n_ct > LATE
    assert seq % seg == 0 and seg % 16 == 0 and n_mem % 8 == 0
    assert N_PRE % UNROLL == 0 and (seq // seg - 1) % UNROLL == 0 and seq // seg > 1 + N_PRE
    assert n_heads % 2 == 0 and 2 * d_head == 3 * LANES and 2 * (seg + n_mem) <= LANES
    assert LATE * PLANES * CHUNK // 8 == 3 * inner // LANES

    def feature_major(w):
        return jnp.transpose(w, (1, 2, 0)).reshape(inner, d_model)

    fwd, inv = _dft_constants()
    small = (
        A_mem0.reshape(n_mem, d_model), B_shift_k.T, B_ssm_D, gate_w,
        jnp.asarray(fwd, _BF16), jnp.asarray(inv, _BF16),
    )
    big = (
        A_x.reshape(seq, d_model),
        feature_major(A_Wq), feature_major(A_Wk), feature_major(A_Wv),
        A_Wo.reshape(inner, d_model),
        B_k.reshape(seq, d_model), B_v.reshape(seq, d_model), B_ssm_k,
    )
    any_spec = pl.BlockSpec(memory_space=pl.ANY)
    spectra = pltpu.VMEM((n_chunks, LATE * PLANES * CHUNK, LANES), _F32)
    out = pl.pallas_call(
        functools.partial(_kernel, seg=seg, n_heads=n_heads, d_head=d_head),
        out_shape=jax.ShapeDtypeStruct((seq, d_model), A_x.dtype),
        in_specs=[any_spec] * (len(big) + len(small)),
        out_specs=any_spec,
        scratch_shapes=[pltpu.VMEM(a.shape, a.dtype) for a in small] + [
            pltpu.VMEM((seq, d_model), _BF16),
            pltpu.VMEM((n_ct, seq, LANES), _BF16),
            pltpu.VMEM((n_ct, seq, LANES), _BF16),
            pltpu.VMEM((n_ct, LANES, seq), _BF16),
            pltpu.VMEM((4, inner, d_model), _BF16),
            pltpu.VMEM((3, inner // LANES, d_model // 2, LANES), jnp.int32),
            pltpu.VMEM((inner // LANES, LANES // 2, d_model), jnp.int32),
            pltpu.VMEM((seq + 8, LANES), _F32),
            spectra,
            spectra,
            pltpu.VMEM((n_ct, seq, LANES), _F32),
            pltpu.VMEM((3, inner // LANES, N_PRE * PRE, LANES), _F32),
            pltpu.VMEM(((seg + n_mem + N_PRE * PRE) // 2, d_model), jnp.int32),
            pltpu.VMEM((seq, d_model), A_x.dtype),
            pltpu.VMEM((8, LANES), jnp.int32),
            pltpu.SemaphoreType.DMA((len(small),)),
            pltpu.SemaphoreType.DMA((3, n_ct)),
            pltpu.SemaphoreType.DMA((4, n_heads // 2)),
            pltpu.SemaphoreType.DMA((2,)),
            pltpu.SemaphoreType.DMA(()),
        ],
        compiler_params=pltpu.CompilerParams(vmem_limit_bytes=122 * 1024 * 1024),
        name="gated_mix_rmt_h3",
    )(*big, *small)
    return out.reshape(batch, seq, d_model)
```

```python
import functools

import jax
import jax.numpy as jnp
import numpy as np
from jax import lax
import jax.experimental.pallas as pl
import jax.experimental.pallas.tpu as pltpu

LANES = 128
CHUNK = 128
PLANES = 3
LATE = 3
UNROLL = 3
PRE = 8
N_PRE = 33
CONV_UNROLL = 4
TIE = 3

LAG_S, LAG_PV, LAG_O = 1, 4, 6

_F32 = jnp.float32
_BF16 = jnp.bfloat16
_NT = (((1,), (1,)), ((), ()))


def _dft_constants():
    w = np.pi * (np.arange(CHUNK, dtype=np.float64) + 0.5) / CHUNK
    t = np.arange(CHUNK, dtype=np.float64)
    ang = w[:, None] * t[None, :]
    fwd = np.concatenate([np.cos(ang), -np.sin(ang)], axis=0)
    inv = np.concatenate([np.cos(ang.T), -np.sin(ang.T)], axis=1) / CHUNK
    return fwd.astype(np.float32), inv.astype(np.float32)


def _dot(a, b):
    return jnp.dot(a, b, preferred_element_type=_F32)


def _dot_nt(a, b):
    return lax.dot_general(a, b, _NT, preferred_element_type=_F32)


def _rows(start, size, align):
    return pl.ds(start if isinstance(start, int) else pl.multiple_of(start, align), size)


def _kernel(
    x_hbm, wq_hbm, wk_hbm, wv_hbm, wo_hbm, k_hbm, v_hbm, ssmk_hbm,
    mem0_hbm, taps_hbm, ssmd_hbm, gate_hbm, fwd_hbm, inv_hbm,
    out_hbm,
    mem0_s, taps_s, ssmd_s, gate_s, fwd_s, inv_s,
    x_s, k_s, v_s, ssmk_s, wt_s, w_s, wo_s, kf_s, xh_s, kh_s, b_s,
    pre_s, h0_s, out_s, ones_s, q_s, kb_s, vb_s, acc_s,
    small_sem, in_sem, w_sem, x_sem, out_sem,
    *, seg, n_heads, d_head,
):
    n_ct, seq, _ = k_s.shape
    d_model = n_ct * LANES
    n_mem = mem0_s.shape[0]
    n_taps = taps_s.shape[0]
    n_chunks = seq // CHUNK
    n_seg = seq // seg
    rows = seg + n_mem
    n_pairs = n_heads // 2
    pair_w = 2 * d_head
    pair_t = pair_w // LANES
    scale = float(d_head) ** -0.5
    x_head = (1 + N_PRE) * seg
    spec = PLANES * CHUNK

    small_copies = [
        pltpu.make_async_copy(src, dst, small_sem.at[i])
        for i, (src, dst) in enumerate((
            (fwd_hbm, fwd_s), (taps_hbm, taps_s), (ssmd_hbm, ssmd_s),
            (inv_hbm, inv_s), (mem0_hbm, mem0_s), (gate_hbm, gate_s)))
    ]

    def act_copies(c):
        cols = _rows(c * LANES, LANES, LANES)
        return (
            pltpu.make_async_copy(ssmk_hbm.at[cols, :], ssmk_s.at[c], in_sem.at[0, c]),
            pltpu.make_async_copy(k_hbm.at[:, cols], k_s.at[c], in_sem.at[1, c]),
            pltpu.make_async_copy(v_hbm.at[:, cols], v_s.at[c], in_sem.at[2, c]),
        )

    def w_copy(m, p):
        src = (wq_hbm, wk_hbm, wv_hbm, wo_hbm)[m]
        r = _rows(p * pair_w, pair_w, pair_w)
        return pltpu.make_async_copy(src.at[r, :], wt_s.at[m, r, :], w_sem.at[m, p])

    def x_copy(j):
        r = pl.ds(0, x_head) if j == 0 else pl.ds(x_head, seq - x_head)
        return pltpu.make_async_copy(x_hbm.at[r, :], x_s.at[r, :], x_sem.at[j])

    def start_weights(lo, hi):
        @pl.loop(lo, hi)
        def _(p):
            for m in range(4):
                w_copy(m, p).start()

    for cp in small_copies:
        cp.start()

    @pl.loop(0, n_ct)
    def _(c):
        for cp in act_copies(c):
            cp.start()

    x_copy(0).start()
    batch = (0, 5 * n_pairs // 16, 9 * n_pairs // 16, n_pairs)
    start_weights(batch[0], batch[1])
    for cp in small_copies:
        cp.wait()

    kf_s[0:8, :] = jnp.zeros((8, LANES), _F32)
    freq = lax.broadcasted_iota(jnp.int32, (CHUNK, LANES), 0)
    sign = jnp.where(freq % 2 == 0, 1.0, -1.0).astype(_F32)
    ssm_d = ssmd_s[...].astype(_F32).reshape(1, d_model)

    def slot(c):
        return pl.ds((c % LATE) * spec, spec)

    def filter_spectrum(c, j):
        kf = _dot_nt(fwd_s[...], ssmk_s[c, :, j * CHUNK:(j + 1) * CHUNK])
        kr, ki = kf[:CHUNK], kf[CHUNK:]
        kh_s[j, slot(c), :] = jnp.concatenate([kr, ki - kr, kr + ki], axis=0)

    def signal_spectrum(c, j):
        cols = slice(c * LANES, (c + 1) * LANES)
        taps = taps_s[:, cols].astype(_F32)
        r0 = j * CHUNK
        ks = kf_s[pl.ds(r0 + 8, CHUNK), :] * taps[0:1, :]
        for t in range(1, n_taps):
            ks = ks + kf_s[pl.ds(r0 + 8 - t, CHUNK), :] * taps[t:t + 1, :]
        kv = (ks * v_s[c, pl.ds(r0, CHUNK), :].astype(_F32)).astype(_BF16)
        b_s[c, pl.ds(r0, CHUNK), :] = kv.astype(_F32) * ssm_d[:, cols]
        xf = _dot(fwd_s[...], kv)
        xr, xi = xf[:CHUNK], xf[CHUNK:]
        xh_s[j, slot(c), :] = jnp.concatenate([xr + xi, xr, xi], axis=0)

    def tie(value, other):
        return jnp.where(ones_s[...] > 0, value, other)

    def chunk_conv(g, after=None):
        f = _rows(g * 8, 8, 8)
        xs, ks = [], []
        for i in range(n_chunks):
            xs.append(xh_s[i, f, :])
            if i == 0 and after is not None:
                xs[0] = tie(xs[0], after)
            ks.append(kh_s[i, f, :])
            acc = xs[0] * ks[i]
            for j in range(1, i + 1):
                acc = acc + xs[j] * ks[i - j]
            xh_s[i, f, :] = acc
        return acc

    def response(c, i):
        a = xh_s[i, slot(c), :]
        a0, a1, a2 = (a[n * CHUNK:(n + 1) * CHUNK] for n in range(PLANES))
        return a0 - a2, a0 + a1

    def inverse(c, i):
        yr, yi = response(c, i)
        if i > 0:
            pr, pi = response(c, i - 1)
            yr, yi = yr - sign * pi, yi + sign * pr
        yf = jnp.concatenate([yr, yi], axis=0).astype(_BF16)
        b_s[c, i * CHUNK:(i + 1) * CHUNK, :] += _dot(inv_s[...], yf)

    n_early = n_ct - LATE
    for c in range(n_ct):
        filt, key, val = act_copies(c)
        filt.wait()
        if c == 0:
            for j in range(n_chunks):
                filter_spectrum(c, j)
        key.wait()
        val.wait()
        kf_s[8:, :] = k_s[c].astype(_F32)
        for j in range(n_chunks):
            signal_spectrum(c, j)
            if c > 0:
                filter_spectrum(c, j)
            if 0 < c <= n_early:
                inverse(c - 1, j)
        if c < n_early:
            g0 = (c % LATE) * spec // 8

            @pl.loop(g0, g0 + spec // 8, unroll=CONV_UNROLL)
            def _(g):
                chunk_conv(g)

        if c == 1:
            start_weights(batch[1], batch[2])
    start_weights(batch[2], batch[3])
    x_copy(1).start()

    qi = lax.broadcasted_iota(jnp.int32, (rows, 2 * rows), 0)
    col = lax.broadcasted_iota(jnp.int32, (rows, 2 * rows), 1)
    head0 = col < rows
    kj = jnp.where(head0, col, col - rows)
    allowed = (qi >= seg) | (kj >= seg) | (qi >= kj)
    lane = lax.broadcasted_iota(jnp.int32, (rows, LANES), 1)
    low_half = lane < (d_head - LANES)
    zeros = jnp.zeros((rows, LANES), _F32)
    gate_w = gate_s[...].astype(_F32).reshape(1, d_model)

    def block_diag(t):
        top = jnp.concatenate([t[0], jnp.where(low_half, t[1], 0.0), zeros], axis=1)
        bot = jnp.concatenate([zeros, jnp.where(low_half, 0.0, t[1]), t[2]], axis=1)
        return jnp.concatenate([top, bot], axis=0).astype(_BF16)

    def probabilities(q, kb):
        s = jnp.where(allowed, _dot_nt(q, kb) * scale, -1e9)
        m0 = jnp.max(jnp.where(head0, s, -jnp.inf), axis=1, keepdims=True)
        m1 = jnp.max(jnp.where(head0, -jnp.inf, s), axis=1, keepdims=True)
        e = jnp.exp(s - jnp.where(head0, m0, m1))
        l0 = jnp.sum(jnp.where(head0, e, 0.0), axis=1, keepdims=True)
        l1 = jnp.sum(jnp.where(head0, 0.0, e), axis=1, keepdims=True)
        return e / jnp.where(head0, l0, l1)

    def out_tile(o, p, c):
        o = jnp.concatenate([o[seg:], o[:seg]], axis=0)
        w = jnp.concatenate(
            [wo_s[p * pair_t + t, :, c * LANES:(c + 1) * LANES]
             for t in range(pair_t)], axis=0)
        return _dot(o, pltpu.bitcast(w, _BF16))

    def out_project(o, p):
        return [out_tile(o, p, c) for c in range(n_ct)]

    def add(acc, ys):
        return [a + y for a, y in zip(acc, ys)]

    def finish(s, xs, acc):
        r = _rows(s * seg, seg, seg)
        a = jnp.concatenate(acc, axis=1)
        g = jax.nn.sigmoid(jnp.sum(xs * gate_w, axis=1, keepdims=True))
        b = xs * jnp.concatenate([b_s[c, r, :] for c in range(n_ct)], axis=1)
        out_s[r, :] = (g * a[n_mem:] + (1.0 - g) * b).astype(out_s.dtype)
        return a[:n_mem]

    x_copy(0).wait()
    xs0 = x_s[0:seg, :].astype(_F32)
    h0_s[...] = pltpu.bitcast(jnp.concatenate(
        [xs0, mem0_s[...].astype(_F32)]
        + [x_s[s * seg:(s + 1) * seg, :].astype(_F32)[seg - PRE:]
           for s in range(1, 1 + N_PRE)], axis=0).astype(_BF16), jnp.int32)

    def staged(m, p, t):
        return wt_s[m, _rows((p * pair_t + t) * LANES, LANES, LANES), :]

    def project_staged(m, p, link):
        ys = []
        for t in range(pair_t):
            w = staged(m, p, t)
            w_s[m, p * pair_t + t] = pltpu.bitcast(w.T, jnp.int32)
            h = h0_s[...]
            if len(link) >= TIE:
                corner = tie(h[:8, :LANES], pltpu.bitcast(link[-TIE], jnp.int32))
                top = jnp.concatenate([corner, h[:8, LANES:]], axis=1)
                h = jnp.concatenate([top, h[8:]], axis=0)
            y = _dot_nt(pltpu.bitcast(h, _BF16), w)
            link.append(chunk_conv((p * 3 + m) * pair_t + t, y[:8]))
            pre_s[m, p * pair_t + t] = y[rows:]
            ys.append(y[:rows])
        return ys

    def repack_wo(p):
        for t in range(pair_t):
            wo_s[p * pair_t + t] = pltpu.bitcast(staged(3, p, t), jnp.int32)

    for m in range(3):
        w_copy(m, 0).wait()
    ones_s[...] = jnp.ones(ones_s.shape, jnp.int32)
    link = []
    q_s[...] = jnp.concatenate(project_staged(0, 0, link), axis=1)
    kb_s[...] = pltpu.bitcast(block_diag(project_staged(1, 0, link)), jnp.int32)
    vb_s[...] = pltpu.bitcast(block_diag(project_staged(2, 0, link)), jnp.int32)
    acc_s[...] = jnp.zeros(acc_s.shape, _F32)

    def first_step(p, carry):
        w_copy(3, p - 1).wait()
        for m in range(3):
            w_copy(m, p).wait()
        repack_wo(p - 1)
        prob = probabilities(q_s[...], pltpu.bitcast(kb_s[...], _BF16))
        link = []
        q_s[...] = jnp.concatenate(project_staged(0, p, link), axis=1)
        o = _dot(prob, pltpu.bitcast(vb_s[...], _BF16))
        kb_s[...] = pltpu.bitcast(block_diag(project_staged(1, p, link)), jnp.int32)
        acc_s[...] += jnp.concatenate(out_project(o, p - 1), axis=1)
        vb_s[...] = pltpu.bitcast(block_diag(project_staged(2, p, link)), jnp.int32)
        return carry

    lax.fori_loop(1, n_pairs, first_step, None)
    prob = probabilities(q_s[...], pltpu.bitcast(kb_s[...], _BF16))
    o = _dot(prob, pltpu.bitcast(vb_s[...], _BF16))
    acc0 = [acc_s[:, c * LANES:(c + 1) * LANES] for c in range(n_ct)]
    for c in range(n_early, n_ct):
        for i in range(n_chunks):
            inverse(c, i)
    w_copy(3, n_pairs - 1).wait()
    repack_wo(n_pairs - 1)
    mem1 = finish(0, xs0, add(acc0, out_project(o, n_pairs - 1)))

    def step(s, mem, has_pre):
        xs = x_s[_rows(s * seg, seg, seg), :].astype(_F32)
        if has_pre:
            h = jnp.concatenate([xs[:seg - PRE], mem], axis=0).astype(_BF16)
        else:
            h = jnp.concatenate([xs, mem], axis=0)

        def project(m, tile):
            y = _dot(h, pltpu.bitcast(w_s[m, tile], _BF16))
            if has_pre:
                early = pre_s[m, tile, _rows((s - 1) * PRE, PRE, PRE), :]
                y = jnp.concatenate([y[:seg - PRE], early, y[seg - PRE:]], axis=0)
            return y

        q, kb, vb, prob, o = {}, {}, {}, {}, {}
        acc = [None] * n_ct

        def emit(p, c):
            if 0 <= p < n_pairs:
                y = out_tile(o[p], p, c)
                acc[c] = y if acc[c] is None else acc[c] + y

        n_proj = 3 * pair_t
        emit_after = {c * n_proj // n_ct: c for c in range(n_ct)} if has_pre else {}
        for p in range(n_pairs + LAG_O):
            ys = []
            for u in range(n_proj):
                if p < n_pairs:
                    ys.append(project(u // pair_t, p * pair_t + u % pair_t))
                if u in emit_after:
                    emit(p - LAG_O, emit_after[u])
            if p < n_pairs:
                q[p] = jnp.concatenate(ys[:pair_t], axis=1)
                kb[p] = block_diag(ys[pair_t:2 * pair_t])
                vb[p] = block_diag(ys[2 * pair_t:])
            if 0 <= p - LAG_S < n_pairs:
                prob[p - LAG_S] = probabilities(q.pop(p - LAG_S), kb.pop(p - LAG_S))
            if 0 <= p - LAG_PV < n_pairs:
                o[p - LAG_PV] = _dot(prob.pop(p - LAG_PV), vb.pop(p - LAG_PV))
            if not has_pre:
                for c in range(n_ct):
                    emit(p - LAG_O, c)
        return finish(s, xs, acc)

    def out_copy(start, size):
        r = _rows(start, size, seg)
        return pltpu.make_async_copy(out_s.at[r, :], out_hbm.at[r, :], out_sem)

    def run(s0, n, has_pre, mem):
        def body(i, mem):
            @pl.when(i > 0)
            def _():
                out_copy((s0 + (i - 1) * UNROLL) * seg, UNROLL * seg).start()

            for u in range(UNROLL):
                mem = step(s0 + i * UNROLL + u, mem, has_pre)
            return mem

        mem = lax.fori_loop(0, n // UNROLL, body, mem)
        out_copy((s0 + n - UNROLL) * seg, UNROLL * seg).start()
        return mem

    out_copy(0, seg).start()
    mem = run(1, N_PRE, True, mem1)
    x_copy(1).wait()
    run(1 + N_PRE, n_seg - 1 - N_PRE, False, mem)
    out_copy(0, seq).wait()


@functools.partial(jax.jit, static_argnames=("A_seg_len",))
def pallas_gated_mix__memory_aug_recurrent_mem_tr__ssm_conv_h3__prompt_kernel(
    A_x: jax.Array,
    A_mem0: jax.Array,
    A_Wq: jax.Array,
    A_Wk: jax.Array,
    A_Wv: jax.Array,
    A_Wo: jax.Array,
    A_seg_len: int,
    B_q: jax.Array,
    B_k: jax.Array,
    B_v: jax.Array,
    B_shift_k: jax.Array,
    B_ssm_k: jax.Array,
    B_ssm_D: jax.Array,
    gate_w: jax.Array,
):
    del B_q
    batch, seq, d_model = A_x.shape
    n_mem = A_mem0.shape[1]
    _, n_heads, d_head = A_Wq.shape
    seg = int(A_seg_len)
    inner = n_heads * d_head
    n_ct = d_model // LANES
    n_chunks = seq // CHUNK
    assert batch == 1 and d_model % LANES == 0 and seq % CHUNK == 0 and n_ct > LATE
    assert seq % seg == 0 and seg % 16 == 0 and n_mem % 8 == 0
    assert N_PRE % UNROLL == 0 and (seq // seg - 1) % UNROLL == 0 and seq // seg > 1 + N_PRE
    assert n_heads % 2 == 0 and 2 * d_head == 3 * LANES and 2 * (seg + n_mem) <= LANES
    assert LATE * PLANES * CHUNK // 8 == 3 * inner // LANES

    def feature_major(w):
        return jnp.transpose(w, (1, 2, 0)).reshape(inner, d_model)

    fwd, inv = _dft_constants()
    small = (
        A_mem0.reshape(n_mem, d_model), B_shift_k.T, B_ssm_D, gate_w,
        fwd.astype(_BF16), inv.astype(_BF16),
    )
    big = (
        A_x.reshape(seq, d_model),
        feature_major(A_Wq), feature_major(A_Wk), feature_major(A_Wv),
        A_Wo.reshape(inner, d_model),
        B_k.reshape(seq, d_model), B_v.reshape(seq, d_model), B_ssm_k,
    )
    any_spec = pl.BlockSpec(memory_space=pl.ANY)
    spectra = pltpu.VMEM((n_chunks, LATE * PLANES * CHUNK, LANES), _F32)
    out = pl.pallas_call(
        functools.partial(_kernel, seg=seg, n_heads=n_heads, d_head=d_head),
        out_shape=jax.ShapeDtypeStruct((seq, d_model), A_x.dtype),
        in_specs=[any_spec] * (len(big) + len(small)),
        out_specs=any_spec,
        scratch_shapes=[pltpu.VMEM(a.shape, a.dtype) for a in small] + [
            pltpu.VMEM((seq, d_model), _BF16),
            pltpu.VMEM((n_ct, seq, LANES), _BF16),
            pltpu.VMEM((n_ct, seq, LANES), _BF16),
            pltpu.VMEM((n_ct, LANES, seq), _BF16),
            pltpu.VMEM((4, inner, d_model), _BF16),
            pltpu.VMEM((3, inner // LANES, d_model // 2, LANES), jnp.int32),
            pltpu.VMEM((inner // LANES, LANES // 2, d_model), jnp.int32),
            pltpu.VMEM((seq + 8, LANES), _F32),
            spectra,
            spectra,
            pltpu.VMEM((n_ct, seq, LANES), _F32),
            pltpu.VMEM((3, inner // LANES, N_PRE * PRE, LANES), _F32),
            pltpu.VMEM(((seg + n_mem + N_PRE * PRE) // 2, d_model), jnp.int32),
            pltpu.VMEM((seq, d_model), A_x.dtype),
            pltpu.VMEM((8, LANES), jnp.int32),
            pltpu.VMEM((seg + n_mem, 2 * d_head), _F32),
            pltpu.VMEM((seg + n_mem, 2 * d_head), jnp.int32),
            pltpu.VMEM((seg + n_mem, 2 * d_head), jnp.int32),
            pltpu.VMEM((seg + n_mem, d_model), _F32),
            pltpu.SemaphoreType.DMA((len(small),)),
            pltpu.SemaphoreType.DMA((3, n_ct)),
            pltpu.SemaphoreType.DMA((4, n_heads // 2)),
            pltpu.SemaphoreType.DMA((2,)),
            pltpu.SemaphoreType.DMA(()),
        ],
        compiler_params=pltpu.CompilerParams(vmem_limit_bytes=122 * 1024 * 1024),
        name="gated_mix_rmt_h3",
    )(*big, *small)
    return out.reshape(batch, seq, d_model)
```
